```python
import jax
import jax.numpy as jnp

def _softmax(x, axis=-1):
    return jax.nn.softmax(x, axis=axis)

def _gelu(x):
    return jax.nn.gelu(x, approximate=True)

def _silu(x):
    return jax.nn.silu(x)

def _sigmoid(x):
    return jax.nn.sigmoid(x)

def _layernorm(x, axis=-1, eps=1e-05):
    m = jnp.mean(x, axis=axis, keepdims=True)
    v = jnp.var(x, axis=axis, keepdims=True)
    return (x - m) / jnp.sqrt(v + eps)

def _scatter_add(tgt, idx, src, axis=0):
    return tgt.at[idx].add(src)

def _segment_sum(src, seg, n):
    return jax.ops.segment_sum(src, seg, n)

class _Rng:

    def __init__(self, key):
        self._k = key

    def _next(self):
        self._k, sub = jax.random.split(self._k)
        return sub

    def normal(self, shape):
        return jax.random.normal(self._next(), shape, dtype=jnp.bfloat16)

    def randint(self, lo, hi, shape):
        return jax.random.randint(self._next(), shape, lo, hi, dtype=jnp.int32)

    def uniform(self, shape, lo=0.0, hi=1.0):
        return jax.random.uniform(self._next(), shape, jnp.bfloat16, lo, hi)

    def permutation(self, n):
        return jax.random.permutation(self._next(), n)
kernel_name = 'standalone__conformer_conv_module__speech'

def setup_inputs():
    _rng = _Rng(jax.random.key(int.from_bytes(__import__("os").urandom(4), "little")))
    _w = lambda a: (lambda t: t.astype(jnp.bfloat16) if jnp.issubdtype(t.dtype, jnp.floating) else t)(jnp.asarray(a))
    B, T, D, K = (2, 16000, 256, 31)
    return {'x': _w((lambda *s: _rng.normal(s) * 0.05)(B, T, D)), 'w_pw1': _w((lambda *s: _rng.normal(s) * 0.05)(D, 2 * D)), 'dw': _w((lambda *s: _rng.normal(s) * 0.05)(K, D)), 'w_pw2': _w((lambda *s: _rng.normal(s) * 0.05)(D, D))}

def reference(x, w_pw1, dw, w_pw2):
    B, T, D = x.shape
    K = dw.shape[0]
    h = x @ w_pw1
    a, b = (h[..., :D].copy(), h[..., D:].copy())
    h = a * _sigmoid(b)
    pad = K // 2
    hp = jnp.pad(h, ((0, 0), (pad, pad), (0, 0)))
    out = jnp.zeros_like(h)
    for i in range(K):
        out = out + hp[:, i:i + T, :] * dw[i][None, None, :]
    return _silu(out) @ w_pw2
```

```python
import jax
import jax.numpy as jnp
import jax.experimental.pallas as pl
import jax.experimental.pallas.tpu as pltpu

L = 100
R = 8 * L
N = L // 4
KL = 8
GAP = 16
F32 = jnp.float32


def _split(h):
    e, o = h[0::2], h[1::2]
    return [e, [a + b for a, b in zip(e, o)], o]


@jax.jit
def pallas_standalone__conformer_conv_module__speech_kernel(x, w_pw1, dw, w_pw2):
    B, T, D = x.shape
    K = dw.shape[0]
    assert D == 256 and K == 31 and T % R == 0
    NB = T // R
    NT = B * NB

    def kernel(x_hbm, w1, dw_ref, w2, o_hbm, xs, os_, g, wt, m, u, isem, osem):
        def in_copy(i):
            r = pl.ds(pl.multiple_of(i * R, R), R)
            return pltpu.make_async_copy(x_hbm.at[r], xs.at[r], isem.at[i])

        def out_copy(i):
            r = pl.ds(pl.multiple_of(i * R, R), R)
            return pltpu.make_async_copy(os_.at[r], o_hbm.at[r], osem.at[i])

        for i in range(NT):
            in_copy(i).start()

        dwf = dw_ref[...].astype(F32)
        for h in range(2):
            taps = [jnp.broadcast_to(dwf[k:k + 1, h * 128:(h + 1) * 128], (8, 128))
                    for k in range(K)] + [jnp.zeros((8, 128), F32)]
            for t, f in enumerate(_split(taps)):
                for s, ff in enumerate(_split(f)):
                    for k in range(KL):
                        wt[((h * 3 + t) * 3 + s) * KL + k] = ff[k]
            for b in range(B + 1):
                g[h, pl.ds(b * (T + GAP), GAP), :] = jnp.zeros((GAP, 128), F32)
        m[...] = jnp.zeros(m.shape, F32)

        def gbase(i):
            return i * R + GAP * (1 + i // NB)

        def sigmoid(v):
            return 0.5 * jnp.tanh(0.5 * v) + 0.5

        def stage_a(i, c, h):
            xv = xs[pl.ds(pl.multiple_of(i * R + c * (R // 2), 16), R // 2), :]
            a = jnp.dot(xv, w1[:, h * 128:(h + 1) * 128], preferred_element_type=F32)
            b = jnp.dot(xv, w1[:, D + h * 128:D + (h + 1) * 128], preferred_element_type=F32)
            g[h, pl.ds(pl.multiple_of(gbase(i) + c * (R // 2), 8), R // 2), :] = a * sigmoid(b)

        def stage_b(i, h, t):
            base = gbase(i) - K // 2
            p = i % 2

            def xl(j):
                return g[h, pl.ds(base + j, 8, stride=L), :]

            def top(j):
                return xl(2 * j + 1) if t == 1 else xl(2 * j + t) - xl(2 * j + 1)

            w = [[wt[((h * 3 + t) * 3 + s) * KL + k] for k in range(KL)] for s in range(3)]
            win = [[], [], []]
            prev = top(0)
            for j in range(N + KL - 1):
                mid, nxt = top(2 * j + 1), top(2 * j + 2)
                for s, v in enumerate((prev - mid, mid, nxt - mid)):
                    win[s].append(v)
                prev = nxt
                o = j - (KL - 1)
                if o >= 0:
                    r = []
                    for s in range(3):
                        acc = win[s][o] * w[s][0]
                        for k in range(1, KL):
                            acc = acc + win[s][o + k] * w[s][k]
                        r.append(acc)
                    m[p, h * 3 + t, 2 * o] = r[0] + r[1]
                    m[p, h * 3 + t, 2 * o + 1] = r[1] + r[2]

        def stage_c(i, c):
            p = i % 2
            cols = []
            for h in range(2):
                rows = []
                for j in range(c * N, (c + 1) * N):
                    m0, m1, m2 = (m[p, h * 3 + t, j] for t in range(3))
                    rows += [m0 + m1, m1 + m2]
                cols.append(jnp.concatenate(rows, axis=0))
            y = 0.5 * jnp.concatenate(cols, axis=1)
            y = (y * jnp.tanh(y) + y).astype(jnp.bfloat16)
            z = jnp.dot(y, w2[...], preferred_element_type=F32)
            for h in range(2):
                for j in range(2 * N):
                    u[h, pl.ds(c * 2 * N + j, 8, stride=L), :] = (
                        z[8 * j:8 * j + 8, h * 128:(h + 1) * 128])

        def flush(i):
            r = pl.ds(pl.multiple_of(i * R, R), R)
            for h in range(2):
                os_[r, h * 128:(h + 1) * 128] = u[h].astype(jnp.bfloat16)

        def pro(i, _):
            in_copy(i).wait()
            for c in range(2):
                for h in range(2):
                    stage_a(i, c, h)
        jax.lax.fori_loop(0, 2, pro, None)

        def body(i, _):
            ia = jnp.minimum(i + 2, NT - 1)
            ic = jnp.maximum(i - 1, 0)

            @pl.when(i + 2 < NT)
            def _():
                in_copy(i + 2).wait()

            for q in range(6):
                @pl.when(i < NT + q)
                def _():
                    stage_b(i, q // 3, q % 3)
                    if q < 2:
                        stage_c(ic, q)
                    else:
                        stage_a(ia, q % 2, (q - 2) // 2)
                    if q == 2:
                        flush(ic)

            @pl.when(i > 0)
            def _():
                out_copy(i - 1).start()
        jax.lax.fori_loop(0, NT, body, None)

        stage_c(NT - 1, 0)
        stage_c(NT - 1, 1)
        flush(NT - 1)
        out_copy(NT - 1).start()
        for i in range(NT):
            out_copy(i).wait()

    vm = pl.BlockSpec(memory_space=pltpu.VMEM)
    hbm = pl.BlockSpec(memory_space=pl.ANY)
    out = pl.pallas_call(
        kernel,
        in_specs=[hbm, vm, vm, vm],
        out_specs=hbm,
        out_shape=jax.ShapeDtypeStruct((B * T, D), x.dtype),
        scratch_shapes=[
            pltpu.VMEM((B * T, D), jnp.bfloat16),
            pltpu.VMEM((B * T, D), jnp.bfloat16),
            pltpu.VMEM((2, B * (T + GAP) + GAP, 128), F32),
            pltpu.VMEM((18 * KL, 8, 128), F32),
            pltpu.VMEM((2, 6, 2 * N, 8, 128), F32),
            pltpu.VMEM((2, R, 128), F32),
            pltpu.SemaphoreType.DMA((NT,)),
            pltpu.SemaphoreType.DMA((NT,)),
        ],
        compiler_params=pltpu.CompilerParams(vmem_limit_bytes=100 * 1024 * 1024),
    )(x.reshape(B * T, D), w_pw1, dw, w_pw2)
    return out.reshape(B, T, D)
```

```python
import jax
import jax.numpy as jnp
import jax.experimental.pallas as pl
import jax.experimental.pallas.tpu as pltpu

L = 100
R = 8 * L
N = L // 4
KL = 8
GAP = 16
F32 = jnp.float32
J0 = 0
PC = 10


def run(fs):
    for f in fs:
        f()


def _split(h):
    e, o = h[0::2], h[1::2]
    return [e, [a + b for a, b in zip(e, o)], o]


@jax.jit
def pallas_standalone__conformer_conv_module__speech_kernel(x, w_pw1, dw, w_pw2):
    B, T, D = x.shape
    K = dw.shape[0]
    assert D == 256 and K == 31 and T % R == 0
    NB = T // R
    NT = B * NB

    def kernel(x_hbm, w1, dw_ref, w2, o_hbm, xs, os_, g, gt, wt, ma, mb, u, gsem, isem, osem, flag):
        def in_copy(i):
            r = pl.ds(pl.multiple_of(i * R, R), R)
            return pltpu.make_async_copy(x_hbm.at[r], xs.at[r], isem.at[i])

        def out_copy(i):
            r = pl.ds(pl.multiple_of(i * R, R), R)
            return pltpu.make_async_copy(os_.at[r], o_hbm.at[r], osem.at[i])

        for i in range(NT):
            in_copy(i).start()

        dwf = dw_ref[...].astype(F32)
        for h in range(2):
            taps = [jnp.broadcast_to(dwf[k:k + 1, h * 128:(h + 1) * 128], (8, 128))
                    for k in range(K)] + [jnp.zeros((8, 128), F32)]
            for t, f in enumerate(_split(taps)):
                for s, ff in enumerate(_split(f)):
                    for k in range(KL):
                        wt[((h * 3 + t) * 3 + s) * KL + k] = ff[k]
            for b in range(B + 1):
                g[h, pl.ds(b * (T + GAP), GAP), :] = jnp.zeros((GAP, 128), F32)
        mb[...] = jnp.zeros(mb.shape, F32)

        def gbase(i):
            return i * R + GAP * (1 + i // NB)

        def g_copy(i):
            return pltpu.make_async_copy(
                gt, g.at[:, pl.ds(pl.multiple_of(gbase(i), 8), R), :], gsem.at[0])

        def sigmoid(v):
            return 0.5 * jnp.tanh(0.5 * v) + 0.5

        def lagged(mm, st):
            n, res = 2 * N // PC, {}
            fs = []
            for p in range(n + 1):
                if p < n:
                    fs.append(lambda p=p: res.__setitem__(p, mm(p)))
                if p > 0:
                    fs.append(lambda p=p: st(p - 1, res[p - 1]))
            gs = [fs[:1]] + [fs[k:k + 2] for k in range(1, len(fs), 2)]
            return [lambda v=v: run(v) for v in gs]

        def stage_a(i, c, h):
            def mm(p):
                xv = xs[pl.ds(pl.multiple_of(i * R + c * (R // 2) + p * 8 * PC, 16), 8 * PC), :]
                return [jnp.dot(xv, w1[:, o + h * 128:o + (h + 1) * 128],
                                preferred_element_type=F32) for o in (0, D)]

            def st(p, ab):
                gt[h, pl.ds(c * (R // 2) + p * 8 * PC, 8 * PC), :] = ab[0] * sigmoid(ab[1])
            return lagged(mm, st)

        def stage_b(i, h, t, m, todo):
            base = gbase(i) - K // 2

            def xl(j):
                return g[h, pl.ds(base + j, 8, stride=L), :]

            def top(j):
                return xl(2 * j + 1) if t == 1 else xl(2 * j + t) - xl(2 * j + 1)

            w = [[wt[((h * 3 + t) * 3 + s) * KL + k] for k in range(KL)] for s in range(3)]
            win = [[], [], []]
            prev = top(0)
            for j in range(N + KL - 1):
                mid, nxt = top(2 * j + 1), top(2 * j + 2)
                for s, v in enumerate((prev - mid, mid, nxt - mid)):
                    win[s].append(v)
                prev = nxt
                o = j - (KL - 1)
                if j >= J0:
                    n, d = len(todo), N + KL - 1 - J0
                    run(todo[-(-(j - J0) * n // d):-(-(j - J0 + 1) * n // d)])
                if o >= 0:
                    r = []
                    for s in range(3):
                        acc = win[s][o] * w[s][0]
                        for k in range(1, KL):
                            acc = acc + win[s][o + k] * w[s][k]
                        r.append(acc)
                    m[h * 3 + t, 2 * o] = r[0] + r[1]
                    m[h * 3 + t, 2 * o + 1] = r[1] + r[2]

        def stage_c(m, c):
            def mm(p):
                cols = []
                for h in range(2):
                    rows = []
                    for j in range(c * N + p * PC // 2, c * N + (p + 1) * PC // 2):
                        m0, m1, m2 = (m[h * 3 + t, j] for t in range(3))
                        rows += [m0 + m1, m1 + m2]
                    cols.append(jnp.concatenate(rows, axis=0))
                y = 0.5 * jnp.concatenate(cols, axis=1)
                y = (y * jnp.tanh(y) + y).astype(jnp.bfloat16)
                return jnp.dot(y, w2[...], preferred_element_type=F32)

            def st(p, z):
                for j in range(PC):
                    for h in range(2):
                        u[h, pl.ds(c * 2 * N + p * PC + j, 8, stride=L), :] = (
                            z[8 * j:8 * j + 8, h * 128:(h + 1) * 128])
            return lagged(mm, st)

        def flush(i):
            def st(j, h):
                r = pl.ds(pl.multiple_of(i * R + 16 * j, 16), 16)
                os_[r, h * 128:(h + 1) * 128] = u[h, 16 * j:16 * j + 16].astype(jnp.bfloat16)
            return [lambda j=j, h=h: st(j, h) for j in range(R // 16) for h in range(2)]

        flag[0] = NT

        def pro(i, _):
            in_copy(i).wait()
            for c in range(2):
                for h in range(2):
                    run(stage_a(i, c, h))
            g_copy(i).start()
            g_copy(i).wait()
        jax.lax.fori_loop(0, 2, pro, None)

        def step(i, mcur, mprev):
            ia = jnp.minimum(i + 2, NT - 1)

            @pl.when(i + 2 < NT)
            def _():
                in_copy(i + 2).wait()

            for q in range(6):
                @pl.when(i < NT + q)
                def _():
                    if q < 4:
                        todo = stage_a(ia, q % 2, q // 2)
                        fl = flush(jnp.maximum(i - 2, 0))[q * N:(q + 1) * N]
                        n = len(todo)
                        todo = [(lambda k=k, f=f: (f(), run(fl[k * N // n:(k + 1) * N // n])))
                                for k, f in enumerate(todo)]
                    else:
                        todo = stage_c(mprev, q - 4)
                    stage_b(i, q // 3, q % 3, mcur, todo)
                if q == 3:
                    pl.when(i + 2 < NT)(lambda: g_copy(ia).start())
                    pl.when(i > 1)(lambda: out_copy(i - 2).start())
            pl.when(i + 2 < NT)(lambda: g_copy(ia).wait())

        def body(k, _):
            step(2 * k, ma, mb)
            step(2 * k + 1, mb, ma)
        u[...] = jnp.zeros(u.shape, F32)
        jax.lax.fori_loop(0, NT // 2, body, None)

        run(flush(NT - 2))
        out_copy(NT - 2).start()
        run(stage_c(mb, 0))
        run(stage_c(mb, 1))
        run(flush(NT - 1))
        out_copy(NT - 1).start()
        for i in range(NT):
            out_copy(i).wait()

    vm = pl.BlockSpec(memory_space=pltpu.VMEM)
    hbm = pl.BlockSpec(memory_space=pl.ANY)
    out = pl.pallas_call(
        kernel,
        in_specs=[hbm, vm, vm, vm],
        out_specs=hbm,
        out_shape=jax.ShapeDtypeStruct((B * T, D), x.dtype),
        scratch_shapes=[
            pltpu.VMEM((B * T, D), jnp.bfloat16),
            pltpu.VMEM((B * T, D), jnp.bfloat16),
            pltpu.VMEM((2, B * (T + GAP) + GAP, 128), F32),
            pltpu.VMEM((2, R, 128), F32),
            pltpu.VMEM((18 * KL, 8, 128), F32),
            pltpu.VMEM((6, 2 * N, 8, 128), F32),
            pltpu.VMEM((6, 2 * N, 8, 128), F32),
            pltpu.VMEM((2, R, 128), F32),
            pltpu.SemaphoreType.DMA((1,)),
            pltpu.SemaphoreType.DMA((NT,)),
            pltpu.SemaphoreType.DMA((NT,)),
            pltpu.SMEM((1,), jnp.int32),
        ],
        compiler_params=pltpu.CompilerParams(vmem_limit_bytes=100 * 1024 * 1024),
    )(x.reshape(B * T, D), w_pw1, dw, w_pw2)
    return out.reshape(B, T, D)
```
